```python
import os as _os
_os.environ.setdefault("JAX_PLATFORMS", "cpu")
import jax
import jax.numpy as jnp

def _softmax(x, axis=-1):
    return jax.nn.softmax(x, axis=axis)
def _gelu(x):
    return jax.nn.gelu(x, approximate=True)
def _silu(x):
    return jax.nn.silu(x)
def _sigmoid(x):
    return jax.nn.sigmoid(x)
def _layernorm(x, axis=-1, eps=1e-5):
    m = jnp.mean(x, axis=axis, keepdims=True)
    v = jnp.var(x, axis=axis, keepdims=True)
    return (x - m) / jnp.sqrt(v + eps)
def _scatter_add(tgt, idx, src, axis=0):
    return tgt.at[idx].add(src)
def _segment_sum(src, seg, n):
    return jax.ops.segment_sum(src, seg, n)
class _Rng:
    def __init__(self, key):
        self._k = key
    def _next(self):
        self._k, sub = jax.random.split(self._k)
        return sub
    def normal(self, shape):
        return jax.random.normal(self._next(), shape, dtype=jnp.bfloat16)
    def randint(self, lo, hi, shape):
        return jax.random.randint(self._next(), shape, lo, hi, dtype=jnp.int32)
    def uniform(self, shape, lo=0.0, hi=1.0):
        return jax.random.uniform(self._next(), shape, jnp.bfloat16, lo, hi)
    def permutation(self, n):
        return jax.random.permutation(self._next(), n)


kernel_name = 'concat_heads__mha_block_cached__mha_block_cached__near_ridge'

def setup_inputs():
    _rng = _Rng(jax.random.key(int.from_bytes(__import__("os").urandom(4), "little")))
    _w = (lambda a: (lambda t: t.astype(jnp.bfloat16) if jnp.issubdtype(t.dtype, jnp.floating) else t)(jnp.asarray(a)))
    def _A_setup():
        B, Sq, D = 8, 144, 640
        H, Sk, Dh = 32, 512, 128
        return {
            "x": _w((lambda *s: _rng.normal(s) * 0.8)(B, Sq, D)),
            "k_cache": _w((lambda *s: _rng.normal(s) * 0.8)(B, H, Sk, Dh)),
            "v_cache": _w((lambda *s: _rng.normal(s) * 0.05)(B, H, Sk, Dh)),
            "wq": _w((lambda *s: _rng.normal(s) * 0.8)(D, H * Dh) * (D ** -0.5)),
            "wo": _w((lambda *s: _rng.normal(s) * 0.05)(H * Dh, D) * ((H * Dh) ** -0.5)),
        }
    _A_in = _A_setup()

    def _B_setup():
        B, Sq, D = 8, 144, 640
        H, Sk, Dh = 32, 512, 128
        return {
            "x": _w((lambda *s: _rng.normal(s) * 0.8)(B, Sq, D)),
            "k_cache": _w((lambda *s: _rng.normal(s) * 0.8)(B, H, Sk, Dh)),
            "v_cache": _w((lambda *s: _rng.normal(s) * 0.05)(B, H, Sk, Dh)),
            "wq": _w((lambda *s: _rng.normal(s) * 0.8)(D, H * Dh) * (D ** -0.5)),
            "wo": _w((lambda *s: _rng.normal(s) * 0.05)(H * Dh, D) * ((H * Dh) ** -0.5)),
        }
    _B_in = _B_setup()

    return {
        "A_x": _A_in["x"],
        "A_k_cache": _A_in["k_cache"],
        "A_v_cache": _A_in["v_cache"],
        "A_wq": _A_in["wq"],
        "A_wo": _A_in["wo"],
        "B_x": _B_in["x"],
        "B_k_cache": _B_in["k_cache"],
        "B_v_cache": _B_in["v_cache"],
        "B_wq": _B_in["wq"],
        "B_wo": _B_in["wo"],
    }

def reference(A_x, A_k_cache, A_v_cache, A_wq, A_wo, B_x, B_k_cache, B_v_cache, B_wq, B_wo):
    def _A_ref(x, k_cache, v_cache, wq, wo):
        B, Sq, D = x.shape
        H, Dh = 32, 128
        q = (lambda x, *d: x.transpose(*d))((x @ wq).reshape(B, Sq, H, Dh), 0, 2, 1, 3)
        scores = jnp.einsum("bhqd,bhkd->bhqk", q, k_cache) * (Dh ** -0.5)
        p = _softmax(scores, axis=-1)
        o = jnp.einsum("bhqk,bhkd->bhqd", p, v_cache)
        return (lambda x, *d: x.transpose(*d))(o, 0, 2, 1, 3).reshape(B, Sq, H * Dh) @ wo

    def _B_ref(x, k_cache, v_cache, wq, wo):
        B, Sq, D = x.shape
        H, Dh = 32, 128
        q = (lambda x, *d: x.transpose(*d))((x @ wq).reshape(B, Sq, H, Dh), 0, 2, 1, 3)
        scores = jnp.einsum("bhqd,bhkd->bhqk", q, k_cache) * (Dh ** -0.5)
        p = _softmax(scores, axis=-1)
        o = jnp.einsum("bhqk,bhkd->bhqd", p, v_cache)
        return (lambda x, *d: x.transpose(*d))(o, 0, 2, 1, 3).reshape(B, Sq, H * Dh) @ wo

    a = _A_ref(A_x, A_k_cache, A_v_cache, A_wq, A_wo)
    b = _B_ref(B_x, B_k_cache, B_v_cache, B_wq, B_wo)
    return jnp.concatenate([a, b], axis=-1)
```

```python
import numpy as np
import jax
import jax.numpy as jnp
from jax import lax
import jax.experimental.pallas as pl
import jax.experimental.pallas.tpu as pltpu

B, SQ, D, H, SK, DH = 8, 144, 640, 32, 512, 128
M = B * SQ

G = 4
LEAD = 4
RING = 4
RING_WQ = 8
XSPLIT = 2
NI = H // G
LOG_NI = NI.bit_length() - 1
NT = 2 * NI

Q_SCALE = float(DH ** -0.5 * np.log2(np.e))

BF16 = jnp.bfloat16
F32 = jnp.float32

ORDER = (("Q", 0), ("S", 0), ("X", 1), ("P", 1), ("O", 3))
ORDER_NO_Q = tuple(o for o in ORDER if o[0] != "Q")


def _mod(g, n):
    return g % n if isinstance(g, int) else lax.bitwise_and(g, n - 1)


def _block_of(g):
    return g // NI if isinstance(g, int) else lax.shift_right_logical(g, LOG_NI)


def _kernel(xa, ka, va, wqa, woa, xb, kb, vb, wqb, wob, out_hbm,
            x_s, k_s, v_s, wq_s, wo_s, q_s, o_s, acc_s, st_s,
            sem_x, sem_k, sem_v, sem_wq, sem_wo, sem_o):
    srcs = ((xa, ka, va, wqa, woa), (xb, kb, vb, wqb, wob))
    GD = G * DH
    XR = M // XSPLIT

    def cp_k(s, j, slot):
        return pltpu.make_async_copy(srcs[s][1].at[:, pl.ds(j * G, G)], k_s.at[slot], sem_k.at[slot])

    def cp_v(s, j, slot):
        return pltpu.make_async_copy(srcs[s][2].at[:, pl.ds(j * G, G)], v_s.at[slot], sem_v.at[slot])

    def cp_wq(s, j, slot):
        return pltpu.make_async_copy(
            srcs[s][3].at[:, pl.ds(pl.multiple_of(j * GD, GD), GD)], wq_s.at[slot], sem_wq.at[slot])

    def cp_wo(s, j, slot):
        return pltpu.make_async_copy(
            srcs[s][4].at[pl.ds(pl.multiple_of(j * GD, GD), GD), :], wo_s.at[slot], sem_wo.at[slot])

    def cp_xa(c):
        return pltpu.make_async_copy(xa.at[pl.ds(c * XR, XR)], x_s.at[0, pl.ds(c * XR, XR)], sem_x.at[c])

    def cp_xb():
        return pltpu.make_async_copy(xb, x_s.at[1], sem_x.at[XSPLIT])

    def cp_out_a():
        return pltpu.make_async_copy(st_s.at[0], out_hbm.at[:, pl.ds(0, D)], sem_o.at[B])

    def cp_out_b(b):
        return pltpu.make_async_copy(
            st_s.at[1, pl.ds(b * SQ, SQ), :], out_hbm.at[pl.ds(b * SQ, SQ), pl.ds(D, D)], sem_o.at[b])

    def prefetch(cp, g, slot):
        if isinstance(g, int):
            if g < NT:
                cp(g // NI, g % NI, slot).start()
            return

        @pl.when(g < NI)
        def _():
            cp(0, g, slot).start()

        @pl.when(jnp.logical_and(g >= NI, g < NT))
        def _():
            cp(1, g - NI, slot).start()

    def q_proj(dst, n, b, j0, j1):
        c = slice(j0 * DH, j1 * DH)
        q = jnp.dot(x_s[_block_of(n), pl.ds(b * SQ, SQ), :], wq_s[_mod(n, RING_WQ), :, c],
                    preferred_element_type=F32)
        dst[b, :, c] = (q * Q_SCALE).astype(BF16)

    one = pl.program_id(0) + 1

    def in_order(fn):
        def body_(i, c):
            fn()
            return c
        lax.fori_loop(0, one, body_, 0)

    in_order(lambda: (cp_xa(0).start(), prefetch(cp_wq, 0, 0)))
    if XSPLIT > 1:
        in_order(lambda: [cp_xa(c).start() for c in range(1, XSPLIT)])
    in_order(lambda: [prefetch(cp_wq, n, n % RING_WQ) for n in range(1, LEAD)])
    for g0 in range(RING):
        in_order(lambda: (prefetch(cp_k, g0, g0), prefetch(cp_v, g0, g0), prefetch(cp_wo, g0, g0),
                          prefetch(cp_wq, g0 + LEAD, (g0 + LEAD) % RING_WQ)))
    acc_s[...] = jnp.zeros_like(acc_s)

    cp_wq(0, 0, 0).wait()
    for c in range(XSPLIT):
        cp_xa(c).wait()
        for b in range(c * B // XSPLIT, (c + 1) * B // XSPLIT):
            q_proj(q_s.at[0], 0, b, 0, G)

    def q_prologue(n, carry):
        cp_wq(0, 0, _mod(n, RING_WQ)).wait()
        for b in range(B):
            q_proj(q_s.at[n], n, b, 0, G)
        return carry

    lax.fori_loop(1, LEAD, q_prologue, 0)

    def iteration(g, with_q, last):
        s, slot = _block_of(g), _mod(g, RING)
        cp_k(0, 0, slot).wait()
        cp_v(0, 0, slot).wait()
        cp_wo(0, 0, slot).wait()
        if with_q:
            cp_wq(0, 0, _mod(g + LEAD, RING_WQ)).wait()

            @pl.when(g == 0)
            def _():
                cp_xb().start()

            @pl.when(g == NI - LEAD)
            def _():
                cp_xb().wait()

            q_win = q_s.at[pl.ds(g, LEAD + 1)]
            q_rd, q_wr = q_win.at[0], q_win.at[LEAD]
        else:
            q_rd = q_s.at[g]
        if last:
            st_s[0] = acc_s[0].astype(BF16)
            cp_out_a().start()

        live = {}

        def stage_q(b, j):
            q_proj(q_wr, g + LEAD, b, j, j + 1)

        def stage_s(b, j):
            live["s", b, j] = lax.dot_general(
                q_rd[b, :, j * DH:(j + 1) * DH], k_s[slot, b, j],
                (((1,), (1,)), ((), ())), preferred_element_type=F32)

        def stage_x(b, j):
            sc = live.pop(("s", b, j))
            m = jnp.max(sc, axis=-1, keepdims=True)
            p = jnp.exp2(sc - m)
            l = jnp.sum(p, axis=-1, keepdims=True)
            r0 = pl.reciprocal(l, approx=True)
            live["r", b, j] = r0 * (2.0 - l * r0)
            live["p", b, j] = p.astype(BF16)

        def stage_p(b, j):
            o = jnp.dot(live.pop(("p", b, j)), v_s[slot, b, j], preferred_element_type=F32)
            o_s[b, :, j * DH:(j + 1) * DH] = (o * live.pop(("r", b, j))).astype(BF16)

        def stage_o(b, j):
            c = slice(j * DH, (j + 1) * DH)
            rows = pl.ds(b * SQ, SQ)
            d = jnp.dot(o_s[b, :, c], wo_s[slot, c, :], preferred_element_type=F32)
            if last and j == G - 1:
                st_s[1, rows, :] = (acc_s[1, rows, :] + d).astype(BF16)
                cp_out_b(b).start()
            else:
                acc_s[s, rows, :] += d

        stages = {"Q": stage_q, "S": stage_s, "X": stage_x, "P": stage_p, "O": stage_o}
        order = ORDER if with_q else ORDER_NO_Q
        units = [(b, j) for b in range(B) for j in range(G)]
        for t in range(len(units) + max(d for _, d in order)):
            for name, delay in order:
                if 0 <= t - delay < len(units):
                    stages[name](*units[t - delay])

        if not last:
            prefetch(cp_k, g + RING, slot)
            prefetch(cp_v, g + RING, slot)
            prefetch(cp_wo, g + RING, slot)
            if with_q:
                prefetch(cp_wq, g + LEAD + RING, _mod(g + LEAD + RING, RING_WQ))

    def loop_main(g, carry):
        iteration(g, True, False)
        return carry

    def loop_tail(g, carry):
        iteration(g, False, False)
        return carry

    lax.fori_loop(0, NT - LEAD, loop_main, 0)
    lax.fori_loop(NT - LEAD, NT - 1, loop_tail, 0)
    iteration(NT - 1, False, True)

    cp_out_a().wait()
    for b in range(B):
        cp_out_b(b).wait()


@jax.jit
def pallas_concat_heads__mha_block_cached__mha_block_cached__near_ridge_kernel(
    A_x: jax.Array,
    A_k_cache: jax.Array,
    A_v_cache: jax.Array,
    A_wq: jax.Array,
    A_wo: jax.Array,
    B_x: jax.Array,
    B_k_cache: jax.Array,
    B_v_cache: jax.Array,
    B_wq: jax.Array,
    B_wo: jax.Array,
):
    hbm = pl.BlockSpec(memory_space=pl.ANY)
    out = pl.pallas_call(
        _kernel,
        grid=(1,),
        in_specs=[hbm] * 10,
        out_specs=hbm,
        out_shape=jax.ShapeDtypeStruct((M, 2 * D), BF16),
        scratch_shapes=[
            pltpu.VMEM((2, M, D), BF16),
            pltpu.VMEM((RING, B, G, SK, DH), BF16),
            pltpu.VMEM((RING, B, G, SK, DH), BF16),
            pltpu.VMEM((RING_WQ, D, G * DH), BF16),
            pltpu.VMEM((RING, G * DH, D), BF16),
            pltpu.VMEM((NT, B, SQ, G * DH), BF16),
            pltpu.VMEM((B, SQ, G * DH), BF16),
            pltpu.VMEM((2, M, D), F32),
            pltpu.VMEM((2, M, D), BF16),
            pltpu.SemaphoreType.DMA((XSPLIT + 1,)),
            pltpu.SemaphoreType.DMA((RING,)),
            pltpu.SemaphoreType.DMA((RING,)),
            pltpu.SemaphoreType.DMA((RING_WQ,)),
            pltpu.SemaphoreType.DMA((RING,)),
            pltpu.SemaphoreType.DMA((B + 1,)),
        ],
        compiler_params=pltpu.CompilerParams(
            dimension_semantics=("arbitrary",),
            vmem_limit_bytes=100 * 1024 * 1024,
        ),
    )(A_x.reshape(M, D), A_k_cache, A_v_cache, A_wq, A_wo,
      B_x.reshape(M, D), B_k_cache, B_v_cache, B_wq, B_wo)
    return out.reshape(B, SQ, 2 * D)
```

```python
import numpy as np
import jax
import jax.numpy as jnp
from jax import lax
import jax.experimental.pallas as pl
import jax.experimental.pallas.tpu as pltpu

B, SQ, D, H, SK, DH = 8, 144, 640, 32, 512, 128
M = B * SQ

G = 4
GD = G * DH
LEAD = 5
RING = 4
NI = H // G
LOG_NI = NI.bit_length() - 1
NT = 2 * NI

Q_SCALE = float(DH ** -0.5 * np.log2(np.e))

BF16 = jnp.bfloat16
F32 = jnp.float32

PROLOGUE = (
    ((0, 1), (0,), ((0, 0, 1),)),
    ((1, 3), (), ((0, 1, 3),)),
    ((3, 6), (), ((0, 3, 6),)),
    ((6, 8), (1,), ((0, 6, 8), (1, 0, 8))),
    (None, (2, 3, 4), ((2, 0, 8), (3, 0, 8), (4, 0, 8))),
)

ORDER_MAIN = (("q", 0), ("o", 4), ("s", 0), ("x", 1), ("p", 1))
ORDER_TAIL = (("s", 0), ("o", 5), ("x", 1), ("p", 2))


def _kernel(xa, ka, va, wqa, woa, xb, kb, vb, wqb, wob, out_hbm,
            x_s, k_s, v_s, wq_s, wo_s, q_s, o_s, acc_s, st_s,
            sem_ring, sem_pro, sem_xb, sem_out):
    srcs = ((xa, ka, va, wqa, woa), (xb, kb, vb, wqb, wob))

    def cp_k(s, j, slot, sem):
        return pltpu.make_async_copy(srcs[s][1].at[:, pl.ds(j * G, G)], k_s.at[slot], sem)

    def cp_v(s, j, slot, sem):
        return pltpu.make_async_copy(srcs[s][2].at[:, pl.ds(j * G, G)], v_s.at[slot], sem)

    def cp_wq(s, j, slot, sem):
        return pltpu.make_async_copy(
            srcs[s][3].at[:, pl.ds(pl.multiple_of(j * GD, GD), GD)], wq_s.at[slot], sem)

    def cp_wo(s, j, slot, sem):
        return pltpu.make_async_copy(
            srcs[s][4].at[pl.ds(pl.multiple_of(j * GD, GD), GD), :], wo_s.at[slot], sem)

    def cp_xa(b0, b1, sem):
        rows = pl.ds(b0 * SQ, (b1 - b0) * SQ)
        return pltpu.make_async_copy(xa.at[rows], x_s.at[0, rows], sem)

    def cp_xb():
        return pltpu.make_async_copy(xb, x_s.at[1], sem_xb.at[0])

    def cp_out_a():
        return pltpu.make_async_copy(st_s.at[0], out_hbm.at[:, pl.ds(0, D)], sem_out.at[0])

    def cp_out_b(b):
        rows = pl.ds(b * SQ, SQ)
        return pltpu.make_async_copy(st_s.at[1, rows, :], out_hbm.at[rows, pl.ds(D, D)], sem_out.at[0])

    def prefetch(cp, n, slot, sem):
        if isinstance(n, int):
            if n < NT:
                cp(n // NI, n % NI, slot, sem).start()
            return

        @pl.when(n < NI)
        def _():
            cp(0, n, slot, sem).start()

        @pl.when(jnp.logical_and(n >= NI, n < NT))
        def _():
            cp(1, n - NI, slot, sem).start()

    def prefetch_group(g, slot, with_wq):
        sem = sem_ring.at[slot]
        prefetch(cp_k, g, slot, sem)
        prefetch(cp_v, g, slot, sem)
        prefetch(cp_wo, g, slot, sem)
        if with_wq:
            prefetch(cp_wq, g + LEAD, g + LEAD, sem)

    def block_of(n):
        return n // NI if isinstance(n, int) else lax.shift_right_logical(n, LOG_NI)

    def q_proj(dst, n, b, j0, j1):
        cols = slice(j0 * DH, j1 * DH)
        q = jnp.dot(x_s[block_of(n), pl.ds(b * SQ, SQ), :], wq_s[n, :, cols], preferred_element_type=F32)
        dst[b, :, cols] = (q * Q_SCALE).astype(BF16)

    one = pl.program_id(0) + 1

    def in_order(fn):
        def body_(i, carry):
            fn()
            return carry
        lax.fori_loop(0, one, body_, 0)

    def prologue_copies(i):
        x_range, wq_groups, _ = PROLOGUE[i]
        cps = [cp_wq(0, n, n, sem_pro.at[i]) for n in wq_groups]
        if x_range is not None:
            cps.append(cp_xa(x_range[0], x_range[1], sem_pro.at[i]))
        return cps

    def start_all(cps):
        for c in cps:
            c.start()

    for i in range(len(PROLOGUE)):
        in_order(lambda: start_all(prologue_copies(i)))
    for g0 in range(RING):
        in_order(lambda: prefetch_group(g0, g0, True))
    in_order(lambda: cp_xb().start())

    acc_s[...] = jnp.zeros_like(acc_s)

    for i, (_, _, work) in enumerate(PROLOGUE):
        for c in prologue_copies(i):
            c.wait()
        for n, b0, b1 in work:
            for b in range(b0, b1):
                q_proj(q_s.at[n], n, b, 0, G)

    def iteration(g, with_q):
        slot = lax.bitwise_and(g, RING - 1)
        sem = sem_ring.at[slot]
        cp_k(0, 0, slot, sem).wait()
        cp_v(0, 0, slot, sem).wait()
        cp_wo(0, 0, slot, sem).wait()
        if with_q:
            cp_wq(0, 0, g + LEAD, sem).wait()

            @pl.when(g == NI - LEAD)
            def _():
                cp_xb().wait()

            s = block_of(g)
            q_win = q_s.at[pl.ds(g, LEAD + 1)]
            q_rd, q_wr = q_win.at[0], q_win.at[LEAD]
        else:
            s = 1
            q_rd = q_s.at[g]

        live = {}

        def stage_q(b, j):
            q_proj(q_wr, g + LEAD, b, j, j + 1)

        def stage_s(b, j):
            live["s", b, j] = lax.dot_general(
                q_rd[b, :, j * DH:(j + 1) * DH], k_s[slot, b, j],
                (((1,), (1,)), ((), ())), preferred_element_type=F32)

        def stage_x(b, j):
            sc = live.pop(("s", b, j))
            m = jnp.max(sc, axis=-1, keepdims=True)
            p = jnp.exp2(sc - m)
            l = jnp.sum(p, axis=-1, keepdims=True)
            r0 = pl.reciprocal(l, approx=True)
            live["r", b, j] = r0 * (2.0 - l * r0)
            live["p", b, j] = p.astype(BF16)

        def stage_p(b, j):
            o = jnp.dot(live.pop(("p", b, j)), v_s[slot, b, j], preferred_element_type=F32)
            o_s[b, :, j * DH:(j + 1) * DH] = (o * live.pop(("r", b, j))).astype(BF16)

        def stage_o(b, j):
            if j % 2 == 0:
                return
            cols = slice((j - 1) * DH, (j + 1) * DH)
            rows = pl.ds(b * SQ, SQ)
            new = acc_s[s, rows, :] + jnp.dot(o_s[b, :, cols], wo_s[slot, cols, :],
                                              preferred_element_type=F32)
            if j == G - 1:
                st_s[s, rows, :] = new.astype(BF16)
                if not with_q:
                    @pl.when(g == NT - 1)
                    def _():
                        cp_out_b(b).start()
            acc_s[s, rows, :] = new

        stages = {"q": stage_q, "s": stage_s, "x": stage_x, "p": stage_p, "o": stage_o}
        order = ORDER_MAIN if with_q else ORDER_TAIL
        units = [(b, j) for b in range(B) for j in range(G)]
        for t in range(len(units) + max(d for _, d in order)):
            for name, delay in order:
                if 0 <= t - delay < len(units):
                    stages[name](*units[t - delay])

        prefetch_group(g + RING, slot, with_q)

    def loop_main(g, carry):
        iteration(g, True)
        return carry

    def loop_tail(g, carry):
        iteration(g, False)
        return carry

    lax.fori_loop(0, NT - LEAD, loop_main, 0)
    cp_out_a().start()
    lax.fori_loop(NT - LEAD, NT, loop_tail, 0)

    cp_out_a().wait()
    for b in range(B):
        cp_out_b(b).wait()


@jax.jit
def pallas_concat_heads__mha_block_cached__mha_block_cached__near_ridge_kernel(
    A_x: jax.Array,
    A_k_cache: jax.Array,
    A_v_cache: jax.Array,
    A_wq: jax.Array,
    A_wo: jax.Array,
    B_x: jax.Array,
    B_k_cache: jax.Array,
    B_v_cache: jax.Array,
    B_wq: jax.Array,
    B_wo: jax.Array,
):
    hbm = pl.BlockSpec(memory_space=pl.ANY)
    out = pl.pallas_call(
        _kernel,
        grid=(1,),
        in_specs=[hbm] * 10,
        out_specs=hbm,
        out_shape=jax.ShapeDtypeStruct((M, 2 * D), BF16),
        scratch_shapes=[
            pltpu.VMEM((2, M, D), BF16),
            pltpu.VMEM((RING, B, G, SK, DH), BF16),
            pltpu.VMEM((RING, B, G, SK, DH), BF16),
            pltpu.VMEM((NT, D, GD), BF16),
            pltpu.VMEM((RING, GD, D), BF16),
            pltpu.VMEM((NT, B, SQ, GD), BF16),
            pltpu.VMEM((B, SQ, GD), BF16),
            pltpu.VMEM((2, M, D), F32),
            pltpu.VMEM((2, M, D), BF16),
            pltpu.SemaphoreType.DMA((RING,)),
            pltpu.SemaphoreType.DMA((len(PROLOGUE),)),
            pltpu.SemaphoreType.DMA((1,)),
            pltpu.SemaphoreType.DMA((1,)),
        ],
        compiler_params=pltpu.CompilerParams(
            dimension_semantics=("arbitrary",),
            vmem_limit_bytes=100 * 1024 * 1024,
            disable_bounds_checks=True,
        ),
    )(A_x.reshape(M, D), A_k_cache, A_v_cache, A_wq, A_wo,
      B_x.reshape(M, D), B_k_cache, B_v_cache, B_wq, B_wo)
    return out.reshape(B, SQ, 2 * D)
```

```python
import numpy as np
import jax
import jax.numpy as jnp
from jax import lax
import jax.experimental.pallas as pl
import jax.experimental.pallas.tpu as pltpu

B, SQ, D, H, SK, DH = 8, 144, 640, 32, 512, 128
M = B * SQ

G = 4
GD = G * DH
LEAD = 5
RING = 4
NI = H // G
LOG_NI = NI.bit_length() - 1
NT = 2 * NI

Q_SCALE = float(DH ** -0.5 * np.log2(np.e))

BF16 = jnp.bfloat16
F32 = jnp.float32

PROLOGUE = (
    ((0, 1), ((0, 0, 2),), ((0, 0, 1, 0, 2),)),
    ((1, 3), (), ((0, 1, 3, 0, 2),)),
    (None, ((0, 2, 4),), ((0, 0, 3, 2, 4),)),
    ((3, 6), (), ((0, 3, 6, 0, 4),)),
    ((6, 8), ((1, 0, 4),), ((0, 6, 8, 0, 4), (1, 0, 8, 0, 4))),
    (None, ((2, 0, 4), (3, 0, 4), (4, 0, 4)), ((2, 0, 8, 0, 4), (3, 0, 8, 0, 4), (4, 0, 8, 0, 4))),
)

ORDER_MAIN = (("q", 0), ("o", 4), ("s", 0), ("x", 1), ("p", 1))
ORDER_TAIL = (("s", 0), ("o", 5), ("x", 1), ("p", 2))


assert LEAD <= NI and RING <= NT - LEAD and G % 2 == 0
assert sorted((n, b, j) for _, _, work in PROLOGUE for n, b0, b1, j0, j1 in work
              for b in range(b0, b1) for j in range(j0, j1)) == [
                  (n, b, j) for n in range(LEAD) for b in range(B) for j in range(G)]


def _kernel(xa, ka, va, wqa, woa, xb, kb, vb, wqb, wob, out_hbm,
            x_s, k_s, v_s, wq_s, wo_s, q_s, o_s, acc_s, st_s,
            sem_ring, sem_pro, sem_xb, sem_out):
    srcs = ((xa, ka, va, wqa, woa), (xb, kb, vb, wqb, wob))

    def cp_k(s, j, slot, sem):
        return pltpu.make_async_copy(srcs[s][1].at[:, pl.ds(j * G, G)], k_s.at[slot], sem)

    def cp_v(s, j, slot, sem):
        return pltpu.make_async_copy(srcs[s][2].at[:, pl.ds(j * G, G)], v_s.at[slot], sem)

    def cp_wq(s, j, slot, sem):
        return pltpu.make_async_copy(
            srcs[s][3].at[:, pl.ds(pl.multiple_of(j * GD, GD), GD)], wq_s.at[slot], sem)

    def cp_wqa_piece(n, j0, j1, sem):
        cols = pl.ds(j0 * DH, (j1 - j0) * DH)
        return pltpu.make_async_copy(wqa.at[:, pl.ds(n * GD + j0 * DH, (j1 - j0) * DH)], wq_s.at[n, :, cols], sem)

    def cp_wo(s, j, slot, sem):
        return pltpu.make_async_copy(
            srcs[s][4].at[pl.ds(pl.multiple_of(j * GD, GD), GD), :], wo_s.at[slot], sem)

    def cp_xa(b0, b1, sem):
        rows = pl.ds(b0 * SQ, (b1 - b0) * SQ)
        return pltpu.make_async_copy(xa.at[rows], x_s.at[0, rows], sem)

    def cp_xb():
        return pltpu.make_async_copy(xb, x_s.at[1], sem_xb.at[0])

    def cp_out_a():
        return pltpu.make_async_copy(st_s.at[0], out_hbm.at[:, pl.ds(0, D)], sem_out.at[0])

    def cp_out_b(b):
        rows = pl.ds(b * SQ, SQ)
        return pltpu.make_async_copy(st_s.at[1, rows, :], out_hbm.at[rows, pl.ds(D, D)], sem_out.at[0])

    def prefetch(cp, n, slot, sem):
        if isinstance(n, int):
            if n < NT:
                cp(n // NI, n % NI, slot, sem).start()
            return

        @pl.when(n < NI)
        def _():
            cp(0, n, slot, sem).start()

        @pl.when(jnp.logical_and(n >= NI, n < NT))
        def _():
            cp(1, n - NI, slot, sem).start()

    def prefetch_group(g, slot, with_wq):
        sem = sem_ring.at[slot]
        prefetch(cp_k, g, slot, sem)
        prefetch(cp_v, g, slot, sem)
        prefetch(cp_wo, g, slot, sem)
        if with_wq:
            prefetch(cp_wq, g + LEAD, g + LEAD, sem)

    def block_of(n):
        return n // NI if isinstance(n, int) else lax.shift_right_logical(n, LOG_NI)

    def q_proj(dst, n, b, j0, j1):
        cols = slice(j0 * DH, j1 * DH)
        q = jnp.dot(x_s[block_of(n), pl.ds(b * SQ, SQ), :], wq_s[n, :, cols], preferred_element_type=F32)
        dst[b, :, cols] = (q * Q_SCALE).astype(BF16)

    one = pl.program_id(0) + 1

    def in_order(fn):
        def body_(i, carry):
            fn()
            return carry
        lax.fori_loop(0, one, body_, 0)

    def prologue_copies(i):
        x_range, wq_pieces, _ = PROLOGUE[i]
        cps = [cp_wqa_piece(n, j0, j1, sem_pro.at[i]) for n, j0, j1 in wq_pieces]
        if x_range is not None:
            cps.append(cp_xa(x_range[0], x_range[1], sem_pro.at[i]))
        return cps

    def start_all(cps):
        for c in cps:
            c.start()

    for i in range(len(PROLOGUE)):
        in_order(lambda: start_all(prologue_copies(i)))
    for g0 in range(RING):
        in_order(lambda: prefetch_group(g0, g0, True))
    in_order(lambda: cp_xb().start())

    acc_s[...] = jnp.zeros_like(acc_s)

    for i, (_, _, work) in enumerate(PROLOGUE):
        for c in prologue_copies(i):
            c.wait()
        for n, b0, b1, j0, j1 in work:
            for b in range(b0, b1):
                q_proj(q_s.at[n], n, b, j0, j1)

    def iteration(g, with_q):
        slot = lax.bitwise_and(g, RING - 1)
        sem = sem_ring.at[slot]
        cp_k(0, 0, slot, sem).wait()
        cp_v(0, 0, slot, sem).wait()
        cp_wo(0, 0, slot, sem).wait()
        if with_q:
            cp_wq(0, 0, g + LEAD, sem).wait()

            @pl.when(g == NI - LEAD)
            def _():
                cp_xb().wait()

            s = block_of(g)
            q_win = q_s.at[pl.ds(g, LEAD + 1)]
            q_rd, q_wr = q_win.at[0], q_win.at[LEAD]
        else:
            s = 1
            q_rd = q_s.at[g]

        live = {}

        def stage_q(b, j):
            q_proj(q_wr, g + LEAD, b, j, j + 1)

        def stage_s(b, j):
            live["s", b, j] = lax.dot_general(
                q_rd[b, :, j * DH:(j + 1) * DH], k_s[slot, b, j],
                (((1,), (1,)), ((), ())), preferred_element_type=F32)

        def stage_x(b, j):
            sc = live.pop(("s", b, j))
            m = jnp.max(sc, axis=-1, keepdims=True)
            p = jnp.exp2(sc - m)
            l = jnp.sum(p, axis=-1, keepdims=True)
            r0 = pl.reciprocal(l, approx=True)
            live["r", b, j] = r0 * (2.0 - l * r0)
            live["p", b, j] = p.astype(BF16)

        def stage_p(b, j):
            o = jnp.dot(live.pop(("p", b, j)), v_s[slot, b, j], preferred_element_type=F32)
            o_s[b, :, j * DH:(j + 1) * DH] = (o * live.pop(("r", b, j))).astype(BF16)

        def stage_o(b, j):
            if j % 2 == 0:
                return
            cols = slice((j - 1) * DH, (j + 1) * DH)
            rows = pl.ds(b * SQ, SQ)
            new = acc_s[s, rows, :] + jnp.dot(o_s[b, :, cols], wo_s[slot, cols, :],
                                              preferred_element_type=F32)
            if j == G - 1:
                st_s[s, rows, :] = new.astype(BF16)
                if not with_q:
                    @pl.when(g == NT - 1)
                    def _():
                        cp_out_b(b).start()
            acc_s[s, rows, :] = new

        stages = {"q": stage_q, "s": stage_s, "x": stage_x, "p": stage_p, "o": stage_o}
        order = ORDER_MAIN if with_q else ORDER_TAIL
        units = [(b, j) for b in range(B) for j in range(G)]
        for t in range(len(units) + max(d for _, d in order)):
            for name, delay in order:
                if 0 <= t - delay < len(units):
                    stages[name](*units[t - delay])

        prefetch_group(g + RING, slot, with_q)

    def loop_main(g, carry):
        iteration(g, True)
        return carry

    def loop_tail(g, carry):
        iteration(g, False)
        return carry

    lax.fori_loop(0, NT - LEAD, loop_main, 0)
    cp_out_a().start()
    lax.fori_loop(NT - LEAD, NT, loop_tail, 0)

    cp_out_a().wait()
    for b in range(B):
        cp_out_b(b).wait()


@jax.jit
def pallas_concat_heads__mha_block_cached__mha_block_cached__near_ridge_kernel(
    A_x: jax.Array,
    A_k_cache: jax.Array,
    A_v_cache: jax.Array,
    A_wq: jax.Array,
    A_wo: jax.Array,
    B_x: jax.Array,
    B_k_cache: jax.Array,
    B_v_cache: jax.Array,
    B_wq: jax.Array,
    B_wo: jax.Array,
):
    hbm = pl.BlockSpec(memory_space=pl.ANY)
    out = pl.pallas_call(
        _kernel,
        grid=(1,),
        in_specs=[hbm] * 10,
        out_specs=hbm,
        out_shape=jax.ShapeDtypeStruct((M, 2 * D), BF16),
        scratch_shapes=[
            pltpu.VMEM((2, M, D), BF16),
            pltpu.VMEM((RING, B, G, SK, DH), BF16),
            pltpu.VMEM((RING, B, G, SK, DH), BF16),
            pltpu.VMEM((NT, D, GD), BF16),
            pltpu.VMEM((RING, GD, D), BF16),
            pltpu.VMEM((NT, B, SQ, GD), BF16),
            pltpu.VMEM((B, SQ, GD), BF16),
            pltpu.VMEM((2, M, D), F32),
            pltpu.VMEM((2, M, D), BF16),
            pltpu.SemaphoreType.DMA((RING,)),
            pltpu.SemaphoreType.DMA((len(PROLOGUE),)),
            pltpu.SemaphoreType.DMA((1,)),
            pltpu.SemaphoreType.DMA((1,)),
        ],
        compiler_params=pltpu.CompilerParams(
            dimension_semantics=("arbitrary",),
            vmem_limit_bytes=100 * 1024 * 1024,
            disable_bounds_checks=True,
        ),
    )(A_x.reshape(M, D), A_k_cache, A_v_cache, A_wq, A_wo,
      B_x.reshape(M, D), B_k_cache, B_v_cache, B_wq, B_wo)
    return out.reshape(B, SQ, 2 * D)
```
